```python
import os as _os
_os.environ.setdefault("JAX_PLATFORMS", "cpu")
import jax
import jax.numpy as jnp

def _softmax(x, axis=-1):
    return jax.nn.softmax(x, axis=axis)
def _gelu(x):
    return jax.nn.gelu(x, approximate=True)
def _silu(x):
    return jax.nn.silu(x)
def _sigmoid(x):
    return jax.nn.sigmoid(x)
def _layernorm(x, axis=-1, eps=1e-5):
    m = jnp.mean(x, axis=axis, keepdims=True)
    v = jnp.var(x, axis=axis, keepdims=True)
    return (x - m) / jnp.sqrt(v + eps)
def _scatter_add(tgt, idx, src, axis=0):
    return tgt.at[idx].add(src)
def _segment_sum(src, seg, n):
    return jax.ops.segment_sum(src, seg, n)
class _Rng:
    def __init__(self, key):
        self._k = key
    def _next(self):
        self._k, sub = jax.random.split(self._k)
        return sub
    def normal(self, shape):
        return jax.random.normal(self._next(), shape, dtype=jnp.bfloat16)
    def randint(self, lo, hi, shape):
        return jax.random.randint(self._next(), shape, lo, hi, dtype=jnp.int32)
    def uniform(self, shape, lo=0.0, hi=1.0):
        return jax.random.uniform(self._next(), shape, jnp.bfloat16, lo, hi)
    def permutation(self, n):
        return jax.random.permutation(self._next(), n)


kernel_name = 'recurrent_scan__ssm_conv_s4__mixer_s_mlp__prompt'

def setup_inputs():
    _rng = _Rng(jax.random.key(int.from_bytes(__import__("os").urandom(4), "little")))
    _w = (lambda a: (lambda t: t.astype(jnp.bfloat16) if jnp.issubdtype(t.dtype, jnp.floating) else t)(jnp.asarray(a)))
    def _A_setup():
        B, L, D, N = 1, 2048, 512, 128
        A_re = -jnp.exp((lambda *s: _rng.normal(s) * 0.1)(D, N))
        A_im = jnp.pi * (lambda *s: _rng.normal(s) * 0.1)(D, N)
        B_re = (lambda *s: _rng.normal(s) * 0.1)(D, N)
        B_im = (lambda *s: _rng.normal(s) * 0.1)(D, N)
        C_re = (lambda *s: _rng.normal(s) * 0.1)(D, N)
        C_im = (lambda *s: _rng.normal(s) * 0.1)(D, N)
        log_dt = (lambda *s: _rng.normal(s) * 0.1)(D) * 0.5 - 4.0
        Dskip = (lambda *s: _rng.normal(s) * 0.05)(D)
        return {
            "u": _w((lambda *s: _rng.normal(s) * 0.05)(B, L, D)),
            "A_re": _w(A_re),
            "A_im": _w(A_im),
            "B_re": _w(B_re),
            "B_im": _w(B_im),
            "C_re": _w(C_re),
            "C_im": _w(C_im),
            "log_dt": _w(log_dt),
            "Dskip": _w(Dskip),
        }
    _A_in = _A_setup()

    def _B_setup():
        B, S, D, F = 1, 2048, 512, 1376
        return {
            "x":  _w((lambda *s: _rng.normal(s) * 0.05)(B, S, D)),
            "w1": _w((lambda *s: _rng.normal(s) * 0.8)(D, D) * (D ** -0.5)),
            "w2": _w((lambda *s: _rng.normal(s) * 0.8)(D, D) * (D ** -0.5)),
            "w3": _w((lambda *s: _rng.normal(s) * 0.8)(D, F) * (D ** -0.5)),
            "w4": _w((lambda *s: _rng.normal(s) * 0.8)(F, D) * (F ** -0.5)),
        }
    _B_in = _B_setup()

    return {
        "A_u": _A_in["u"],
        "A_A_re": _A_in["A_re"],
        "A_A_im": _A_in["A_im"],
        "A_B_re": _A_in["B_re"],
        "A_B_im": _A_in["B_im"],
        "A_C_re": _A_in["C_re"],
        "A_C_im": _A_in["C_im"],
        "A_log_dt": _A_in["log_dt"],
        "A_Dskip": _A_in["Dskip"],
        "B_x": _B_in["x"],
        "B_w1": _B_in["w1"],
        "B_w2": _B_in["w2"],
        "B_w3": _B_in["w3"],
        "B_w4": _B_in["w4"],
    }

def reference(A_u, A_A_re, A_A_im, A_B_re, A_B_im, A_C_re, A_C_im, A_log_dt, A_Dskip, B_x, B_w1, B_w2, B_w3, B_w4):
    def _A_ref(u, A_re, A_im, B_re, B_im, C_re, C_im, log_dt, Dskip):
        Bsz, L, D = u.shape
        dt = jnp.exp(log_dt)[:, None]
        A = A_re + 1j * A_im
        Bc = B_re + 1j * B_im
        Cc = C_re + 1j * C_im
        logdA = dt * A
        dB = dt * Bc
        l = (lambda x, dt: x.astype(dt))(jnp.arange(L), A_re.dtype)
        P = jnp.exp(logdA[:, :, None] * l[None, None, :])
        K = jnp.einsum("dn,dnl,dn->dl", Cc, P, dB).real
        L2 = 2 * L
        Kp = jnp.pad(K, ((0, 0), (0, L)))
        up = (lambda x, *d: x.transpose(*d))(u, 0, 2, 1)
        up = jnp.pad(up, ((0, 0), (0, 0), (0, L)))
        Kf = (lambda x, axes=(-2,-1): jnp.fft.rfft2(x.astype(jnp.float32), axes=axes))(Kp[:, None, :], axes=(-2, -1))
        Uf = (lambda x, axes=(-2,-1): jnp.fft.rfft2(x.astype(jnp.float32), axes=axes))(up[:, :, None, :], axes=(-2, -1))
        Yf = Uf * Kf[None, :, :, :]
        y = (lambda x, s, axes=(-2,-1): jnp.fft.irfft2(x, s=s, axes=axes).astype(jnp.bfloat16))(Yf, (1, L2), axes=(-2, -1))[:, :, 0, :L]
        y = (lambda x, *d: x.transpose(*d))(y, 0, 2, 1) + u * Dskip[None, None, :]
        return y

    def _B_ref(x, w1, w2, w3, w4):
        B, S, D = x.shape
        h = _gelu(_layernorm(x, axis=-1) @ w1)
        c = D // 4
        g0 = jnp.pad(h[:, :, 0*c:1*c], ((0, 0), (1, 0), (0, 0)))[:, :S, :]
        g1 = jnp.pad(h[:, :, 1*c:2*c], ((0, 0), (0, 1), (0, 0)))[:, 1:, :]
        g2 = jnp.pad(h[:, :, 2*c:3*c], ((0, 0), (2, 0), (0, 0)))[:, :S, :]
        g3 = jnp.pad(h[:, :, 3*c:   ], ((0, 0), (0, 2), (0, 0)))[:, 2:, :]
        hs = jnp.concatenate([g0, g1, g2, g3], axis=-1) @ w2
        x1 = x + hs
        h2 = _gelu(_layernorm(x1, axis=-1) @ w3) @ w4
        return x1 + h2

    x = A_u
    xn = _layernorm(x, axis=-1)
    s = _A_ref(xn, A_A_re, A_A_im, A_B_re, A_B_im, A_C_re, A_C_im, A_log_dt, A_Dskip)
    g = _silu(_B_ref(xn, B_w1, B_w2, B_w3, B_w4))
    return x + s * g
```

```python
import numpy as np
import jax
import jax.numpy as jnp
from jax import lax
import jax.experimental.pallas as pl
import jax.experimental.pallas.tpu as pltpu

L = 2048
D = 512
N = 128
F = 1376
FP = 1408
MS = 128
ZUNROLL = 2
BK = 128
NB = L // BK
TP = 256
NP = L // TP
EPS = 1e-5
NR = 24
NJ = 32
NV = 656
PITCH = 520
HC = 256
RP = 136
HPAD = 8

bf16 = jnp.bfloat16
f32 = jnp.float32


def _round_positions():
    l = np.arange(L, dtype=np.float32)
    u = l.view(np.uint32).astype(np.uint64)
    u = (u + 0x7FFF + ((u >> 16) & 1)) & 0xFFFF0000
    return u.astype(np.uint32).view(np.float32).astype(np.int64)


def _v_index(r):
    if r <= 256:
        return int(r)
    if r <= 512:
        return 256 + int(r - 256) // 2
    if r <= 1024:
        return 384 + int(r - 512) // 4
    return 512 + int(r - 1024) // 8


_BLK_V0 = [128 * c if c < 2 else
           256 + 64 * (c - 2) if c < 4 else
           384 + 32 * (c - 4) if c < 8 else
           512 + 16 * (c - 8) for c in range(NB)]
_BLK_NV = [128 if c < 2 else 80 if c < 4 else 48 if c < 8 else 32
           for c in range(NB)]
_COARSE = ([(r, r, 8) for r in range(8)]
           + [(256 + 2 * r, 256 + r, 4) for r in range(4)]
           + [(512 + 256 * k + 4 * r, 384 + 64 * k + r, 2)
              for k in range(2) for r in range(2)]
           + [(1024 + 256 * k, 512 + 32 * k, 1) for k in range(4)]
           + [(2048, 640, 1)])


def _constants():
    t = np.arange(BK)[None, :]
    f = np.arange(BK)[:, None]
    th = 2.0 * np.pi * ((t * (2 * f + 1)) % 512) / 512.0
    fwd = np.concatenate([np.cos(th), -np.sin(th)], axis=0)
    inv = np.concatenate([np.cos(th).T, -np.sin(th).T], axis=1) / BK
    rpos = _round_positions()
    sel = []
    for c in (2, 4, 8):
        w = np.zeros((2 * BK, _BLK_NV[c]))
        for tt in range(BK):
            w[:, _v_index(rpos[c * BK + tt]) - _BLK_V0[c]] += fwd[:, tt]
        sel.append(w)
        for c2 in range(c, 2 * c):
            for tt in range(BK):
                assert (_v_index(rpos[c2 * BK + tt]) - _BLK_V0[c2]
                        == _v_index(rpos[c * BK + tt]) - _BLK_V0[c])
    for c2 in range(2):
        for tt in range(BK):
            assert rpos[c2 * BK + tt] == c2 * BK + tt
    return fwd, inv, sel


def _cmul(ar, ai, br, bi):
    return ar * br - ai * bi, ar * bi + ai * br


def _layernorm(x):
    m = jnp.mean(x, axis=-1, keepdims=True)
    xc = x - m
    v = jnp.mean(xc * xc, axis=-1, keepdims=True)
    return xc * lax.rsqrt(v + EPS)


def _gelu(x):
    c1 = 2.0 * float(np.sqrt(2.0 / np.pi))
    u2 = x * (c1 + (c1 * 0.044715) * (x * x))
    return x / (1.0 + jnp.exp(-u2))


def _pk(x):
    return pltpu.bitcast(x, jnp.uint32)


def _upk(x):
    return pltpu.bitcast(x, bf16)


def _dot(a, b):
    return jnp.dot(a, b, preferred_element_type=f32)


def _kernel(x_hbm, are_ref, aim_ref, bre_ref, bim_ref, cre_ref, cim_ref,
            ldt_ref, dsk_ref, w1_hbm, w2_hbm, w3_hbm, w4_hbm,
            fwd_ref, inv_ref, s1_ref, s2_ref, s3_ref,
            out_hbm,
            x_v, w1_v, w2_v, w3_v, w4_v, out_v,
            dt_s, p1_s, p2_s, r_s, kd_s, kf_s, xf_s, xn_s, h_s, z_s, x1_s, ln_s, h3_s, w1_u, w2_u, w3_u, w4_u, pa_s, pb_s,
            flag_s, in_sems, out_sems):
    cp_x = pltpu.make_async_copy(x_hbm.at[0], x_v, in_sems.at[0])
    flag_s[0] = 1

    def wcopies(j, src, dst):
        return [pltpu.make_async_copy(src.at[:, pl.ds(q * 128, 128)],
                                      dst.at[q, pl.ds(0, src.shape[0])],
                                      in_sems.at[1 + 4 * j + q]) for q in range(4)]

    cp_w1 = wcopies(0, w1_hbm, w1_v)
    cp_w2 = wcopies(1, w2_hbm, w2_v)
    cp_w3 = wcopies(2, w3_hbm, w3_v)
    cp_w4 = wcopies(3, w4_hbm, w4_v)
    for cp in [cp_x] + cp_w1 + cp_w2 + cp_w3 + cp_w4:
        cp.start()
    for q in range(4):
        w3_v[q, pl.ds(F, FP - F), :] = jnp.zeros((FP - F, 128), bf16)
        w4_v[q, pl.ds(F, FP - F), :] = jnp.zeros((FP - F, 128), bf16)

    CH = 64
    dt_row = jnp.exp(ldt_ref[...].reshape(1, D).astype(f32)).astype(bf16).astype(f32)
    dt_s[...] = jnp.broadcast_to(dt_row, (N, D)).T

    def gen_powers(ci, carry):
        r0 = pl.multiple_of(ci * CH, CH)
        rows = pl.ds(r0, CH)
        dt = dt_s[rows, :]
        ar = dt * are_ref[rows, :].astype(f32)
        ai = dt * aim_ref[rows, :].astype(f32)
        dbr = dt * bre_ref[rows, :].astype(f32)
        dbi = dt * bim_ref[rows, :].astype(f32)
        cbr, cbi = _cmul(cre_ref[rows, :].astype(f32), cim_ref[rows, :].astype(f32),
                         dbr, dbi)

        def power(m):
            e = jnp.exp(ar * m)
            return e * jnp.cos(ai * m), e * jnp.sin(ai * m)

        def put1(r, v):
            p1_s[0, pl.ds(r * PITCH + r0, CH), :] = v[0]
            p1_s[1, pl.ds(r * PITCH + r0, CH), :] = v[1]

        l1 = power(1.0)
        l2 = _cmul(*l1, *l1)
        l4 = _cmul(*l2, *l2)
        l8 = _cmul(*l4, *l4)
        n1 = l8
        for _ in range(5):
            n1 = _cmul(*n1, *n1)
        q = (cbr, cbi)
        for j in range(NJ):
            p2_s[0, pl.ds(j * PITCH + r0, CH), :] = q[0]
            p2_s[1, pl.ds(j * PITCH + r0, CH), :] = -q[1]
            if j + 1 < NJ:
                q = _cmul(*q, *l8)
        one = jnp.ones_like(ar)
        zero = jnp.zeros_like(ar)
        put1(0, (one, zero))
        put1(1, l1)
        put1(2, l2)
        put1(3, _cmul(*l2, *l1))
        put1(4, l4)
        put1(5, _cmul(*l4, *l1))
        l6 = _cmul(*l4, *l2)
        put1(6, l6)
        put1(7, _cmul(*l6, *l1))
        put1(8, n1)
        put1(9, _cmul(*n1, *l2))
        put1(10, _cmul(*n1, *l4))
        put1(11, _cmul(*n1, *l6))
        n2 = _cmul(*n1, *n1)
        put1(12, n2)
        put1(13, _cmul(*n2, *l4))
        n3 = _cmul(*n2, *n1)
        put1(14, n3)
        put1(15, _cmul(*n3, *l4))
        n4 = _cmul(*n2, *n2)
        put1(16, n4)
        put1(17, _cmul(*n4, *n1))
        put1(18, _cmul(*n4, *n2))
        put1(19, _cmul(*n4, *n3))
        put1(20, _cmul(*n4, *n4))
        for r in range(21, NR):
            put1(r, (zero, zero))
        return carry

    with jax.named_scope('sc_pow'):
        lax.fori_loop(0, D // CH, gen_powers, 0)

    lane_blk = lax.broadcasted_iota(jnp.int32, (NR, 128), 1) // NJ

    def group(g, carry):
        p1 = jnp.concatenate([jnp.concatenate(
            [p1_s[ri, pl.ds(dp * 128 + g, NR, stride=PITCH), :] for dp in range(4)], axis=0)
            for ri in range(2)], axis=1)
        p2 = jnp.concatenate([jnp.concatenate(
            [p2_s[ri, pl.ds(dp * 128 + g, NJ, stride=PITCH), :] for dp in range(4)], axis=0)
            for ri in range(2)], axis=1)
        o = lax.dot_general(p1.astype(bf16), p2.astype(bf16),
                            (((1,), (1,)), ((), ())), preferred_element_type=f32)
        r = jnp.where(lane_blk == 0, o[0:NR],
                      jnp.where(lane_blk == 1, o[NR:2 * NR],
                                jnp.where(lane_blk == 2, o[2 * NR:3 * NR],
                                          o[3 * NR:4 * NR])))
        r_s[pl.ds(g, NR, stride=RP), :] = r
        return carry

    with jax.named_scope('sc_grp'):
        lax.fori_loop(0, 128, group, 0, unroll=4)

    for dp in range(4):
        kd_s[dp, pl.ds(648, 8), :] = jnp.zeros((8, 128), f32)
    for r, (_, v0, st) in enumerate(_COARSE):
        t = r_s[pl.ds(r * RP, 128), :].T
        for dp in range(4):
            slab = t[dp * NJ:(dp + 1) * NJ, :]
            if r == 20:
                kd_s[dp, pl.ds(v0, 8), :] = slab[0:8]
            elif st == 1:
                kd_s[dp, pl.ds(v0, NJ), :] = slab
            else:
                kd_s[dp, pl.ds(v0, NJ, stride=st), :] = slab

    sgn = jnp.where(lax.broadcasted_iota(jnp.int32, (BK, 1), 0) % 2 == 0, 1.0, -1.0)
    for dp in range(4):
        prev = None
        ln_ = pl.ds(dp * 128, 128)
        for c in range(NB):
            w = (fwd_ref if c < 2 else s1_ref if c < 4 else s2_ref if c < 8 else s3_ref)[...]
            kf = _dot(w, kd_s[dp, pl.ds(_BLK_V0[c], _BLK_NV[c]), :].astype(bf16))
            kr, ki = kf[0:BK], kf[BK:2 * BK]
            if prev is None:
                kr2, ki2 = kr, ki
            else:
                kr2, ki2 = kr - sgn * prev[1], ki + sgn * prev[0]
            kf_s[c, dp, 0:BK, :] = kr2
            kf_s[c, dp, BK:2 * BK, :] = ki2
            kf_s[c, dp, 2 * BK:3 * BK, :] = kr2 + ki2
            prev = (kr, ki)

    cp_x.wait()
    for cp in cp_w1:
        cp.wait()
    for q in range(4):
        w1_u[q] = _pk(w1_v[q])
    h_s[pl.ds(0, HPAD), :] = jnp.zeros((HPAD, D), f32)
    h_s[pl.ds(HPAD + L, HPAD), :] = jnp.zeros((HPAD, D), f32)

    def pre_ln(b):
        rows = pl.ds(pl.multiple_of(b * BK, BK), BK)
        xn = _layernorm(x_v[rows, :].astype(f32)).astype(bf16)
        xn_s[rows, :] = xn
        xnn = _layernorm(xn.astype(f32)).astype(bf16)
        for k in range(4):
            pa_s[b % 2, k] = _pk(xn[:, k * 128:(k + 1) * 128])
            pb_s[b % 2, k] = _pk(xnn[:, k * 128:(k + 1) * 128])

    def pre_mm(b):
        r0 = pl.multiple_of(b * BK, BK)
        xnn = jnp.concatenate([_upk(pb_s[b % 2, k]) for k in range(4)], axis=1)
        for q in range(4):
            xf = _dot(fwd_ref[...], _upk(pa_s[b % 2, q]))
            xf_s[b, q, 0:2 * BK, :] = xf
            xf_s[b, q, 2 * BK:3 * BK, :] = xf[0:BK] + xf[BK:2 * BK]
            h = jax.nn.gelu(_dot(xnn, _upk(w1_u[q])), approximate=True)
            h_s[pl.ds(HPAD + r0, BK), pl.ds(q * 128, 128)] = h.astype(bf16).astype(f32)

    def pre(b, carry):
        pre_mm(b)
        pre_ln(jnp.minimum(b + 1, NB - 1))
        return carry

    with jax.named_scope('sc_pre'):
        pre_ln(0)
        lax.fori_loop(0, NB, pre, 0)

    for cp in cp_w2 + cp_w3 + cp_w4:
        cp.wait()
    for q in range(4):
        w2_u[q] = _pk(w2_v[q])
        for j in range(FP // 128):
            w3_u[q, j] = _pk(w3_v[q, pl.ds(j * 128, 128), :])
            w4_u[q, j] = _pk(w4_v[q, pl.ds(j * 128, 128), :])

    out_copies = []
    dsk = dsk_ref[...].reshape(1, D).astype(f32)
    c4 = D // 4
    KB = TP // BK
    ZR = 8
    NI = BK // ZR
    NU = 4 * NI
    NH = FP // 128

    QB = 4

    def zunit(P, u):
        q = u // NI
        r = (u % NI) * ZR
        rs = [pl.ds(pln * BK + r, ZR) for pln in range(3)]
        acc = [None] * QB
        xc = {}
        for c in range(P * QB + QB):
            kk = [kf_s[c, q, rr, :] for rr in rs]
            for k in range(QB):
                b = P * QB + k
                if c > b:
                    continue
                if b - c not in xc:
                    xc[b - c] = [xf_s[b - c, q, rr, :] for rr in rs]
                t = tuple(kv * xv for kv, xv in zip(kk, xc[b - c]))
                acc[k] = t if acc[k] is None else tuple(a + v for a, v in zip(acc[k], t))
        for k in range(QB):
            p1, p2, p3 = acc[k]
            z_s[P * QB + k, q, 0, rs[0], :] = (p1 - p2).astype(bf16)
            z_s[P * QB + k, q, 1, rs[0], :] = (p3 - p1 - p2).astype(bf16)

    def emit_z(mxu_time, upto=None):
        pass

    def zloop(P):
        @pl.when(flag_s[0] == 1)
        def _():
            for u in range(NU):
                zunit(P, u)

    NM = TP // MS
    for p in range(NP):
        r0 = p * TP
        if p % 2 == 0:
            zloop(p // 2)
        for m in range(NM):
            rm = r0 + m * MS
            mr = pl.ds(m * MS, MS)
            mh = pl.ds(m * MS // 2, MS // 2)
            hsft = jnp.concatenate([
                h_s[pl.ds(HPAD + rm - 1, MS), 0 * c4:1 * c4],
                h_s[pl.ds(HPAD + rm + 1, MS), 1 * c4:2 * c4],
                h_s[pl.ds(HPAD + rm - 2, MS), 2 * c4:3 * c4],
                h_s[pl.ds(HPAD + rm + 2, MS), 3 * c4:4 * c4]], axis=1).astype(bf16)
            for q in range(4):
                ln_ = pl.ds(q * 128, 128)
                x1_s[mr, ln_] = (xn_s[pl.ds(rm, MS), ln_].astype(f32)
                                 + _dot(hsft, _upk(w2_u[q])))
                emit_z(4 / NM)
            ln = _layernorm(x1_s[mr, :]).astype(bf16)
            for k in range(4):
                ln_s[k, mh, :] = _pk(ln[:, k * 128:(k + 1) * 128])
        for j in range(NH):
            for m in range(NM):
                mh = pl.ds(m * MS // 2, MS // 2)
                acc = None
                for k in range(4):
                    t = lax.dot_general(_upk(ln_s[k, mh, :]), _upk(w3_u[k, j]),
                                        (((1,), (1,)), ((), ())), preferred_element_type=f32)
                    acc = t if acc is None else acc + t
                h3_s[j, mh, :] = _pk(jax.nn.gelu(acc, approximate=True).astype(bf16))
                emit_z(4 / NM)
        first = True
        for q in range(4):
            ln_ = pl.ds(q * 128, 128)
            for m in range(NM):
                mr = pl.ds(m * MS, MS)
                mh = pl.ds(m * MS // 2, MS // 2)
                rows = pl.ds(r0 + m * MS, MS)
                emit_z(13 / NM, upto=p if first else None)
                first = False
                o2 = x1_s[mr, ln_]
                for j in range(NH):
                    o2 = o2 + _dot(_upk(h3_s[j, mh, :]), _upk(w4_u[q, j]))
                if MS == BK:
                    y = (_dot(inv_ref[0], z_s[p * KB + m, q, 0])
                         + _dot(inv_ref[1], z_s[p * KB + m, q, 1]))
                else:
                    y = jnp.concatenate([_dot(inv_ref[0], z_s[p * KB + k, q, 0])
                                         + _dot(inv_ref[1], z_s[p * KB + k, q, 1])
                                         for k in range(KB)], axis=0)
                hh = 0.5 * o2
                gate = hh + hh * jnp.tanh(hh)
                s = y + xn_s[rows, ln_].astype(f32) * dsk[:, q * 128:(q + 1) * 128]
                res = x_v[rows, ln_].astype(f32) + s * gate
                out_v[rows, ln_] = res.astype(bf16)
        cp = pltpu.make_async_copy(out_v.at[pl.ds(r0, TP), :],
                                   out_hbm.at[0, pl.ds(r0, TP), :], out_sems.at[p])
        cp.start()
        out_copies.append(cp)
    for cp in out_copies:
        cp.wait()


@jax.jit
def pallas_recurrent_scan__ssm_conv_s4__mixer_s_mlp__prompt_kernel(
    A_u: jax.Array,
    A_A_re: jax.Array,
    A_A_im: jax.Array,
    A_B_re: jax.Array,
    A_B_im: jax.Array,
    A_C_re: jax.Array,
    A_C_im: jax.Array,
    A_log_dt: jax.Array,
    A_Dskip: jax.Array,
    B_x: jax.Array,
    B_w1: jax.Array,
    B_w2: jax.Array,
    B_w3: jax.Array,
    B_w4: jax.Array,
):
    assert A_u.shape == (1, L, D) and A_A_re.shape == (D, N)
    assert A_u.dtype == bf16 and A_A_re.dtype == bf16
    assert B_w3.shape == (D, F)
    fwd, inv, sel = _constants()
    inv = np.stack([inv[:, :BK], inv[:, BK:]])
    consts = [jnp.asarray(c, dtype=bf16) for c in (fwd, inv, *sel)]

    vmem = pl.BlockSpec(memory_space=pltpu.VMEM)
    hbm = pl.BlockSpec(memory_space=pltpu.HBM)
    return pl.pallas_call(
        _kernel,
        out_shape=jax.ShapeDtypeStruct((1, L, D), bf16),
        in_specs=[hbm] + [vmem] * 8 + [hbm] * 4 + [vmem] * 5,
        out_specs=hbm,
        scratch_shapes=[
            pltpu.VMEM((L, D), bf16),
            pltpu.VMEM((4, D, 128), bf16),
            pltpu.VMEM((4, D, 128), bf16),
            pltpu.VMEM((4, FP, 128), bf16),
            pltpu.VMEM((4, FP, 128), bf16),
            pltpu.VMEM((L, D), bf16),
            pltpu.VMEM((D, N), f32),
            pltpu.VMEM((2, NR * PITCH, N), f32),
            pltpu.VMEM((2, NJ * PITCH, N), f32),
            pltpu.VMEM((NR * RP, 128), f32),
            pltpu.VMEM((4, NV, 128), f32),
            pltpu.VMEM((NB, 4, 3 * BK, 128), f32),
            pltpu.VMEM((NB, 4, 3 * BK, 128), f32),
            pltpu.VMEM((L, D), bf16),
            pltpu.VMEM((L + 2 * HPAD, D), f32),
            pltpu.VMEM((NB, 4, 2, BK, 128), bf16),
            pltpu.VMEM((TP, D), f32),
            pltpu.VMEM((4, TP // 2, 128), jnp.uint32),
            pltpu.VMEM((FP // 128, TP // 2, 128), jnp.uint32),
            pltpu.VMEM((4, D // 2, 128), jnp.uint32),
            pltpu.VMEM((4, D // 2, 128), jnp.uint32),
            pltpu.VMEM((4, FP // 128, 64, 128), jnp.uint32),
            pltpu.VMEM((4, FP // 128, 64, 128), jnp.uint32),
            pltpu.VMEM((2, 4, 64, 128), jnp.uint32),
            pltpu.VMEM((2, 4, 64, 128), jnp.uint32),
            pltpu.SMEM((1,), jnp.int32),
            pltpu.SemaphoreType.DMA((17,)),
            pltpu.SemaphoreType.DMA((NP,)),
        ],
        compiler_params=pltpu.CompilerParams(vmem_limit_bytes=110 * 1024 * 1024),
    )(A_u, A_A_re, A_A_im, A_B_re, A_B_im, A_C_re, A_C_im,
      A_log_dt, A_Dskip,
      B_w1, B_w2, B_w3.T, B_w4, *consts)
```

```python
import numpy as np
import jax
import jax.numpy as jnp
from jax import lax
import jax.experimental.pallas as pl
import jax.experimental.pallas.tpu as pltpu

L = 2048
D = 512
N = 128
F = 1376
FP = 1408
MS = 128
ZG = 64
PWB = 16
PW0 = 512 - 16 * PWB
BK = 128
NB = L // BK
TP = 256
NP = L // TP
EPS = 1e-5
NR = 24
NJ = 32
NV = 656
PITCH = 520
RP = 136
HPAD = 8

bf16 = jnp.bfloat16
f32 = jnp.float32


def _round_positions():
    l = np.arange(L, dtype=np.float32)
    u = l.view(np.uint32).astype(np.uint64)
    u = (u + 0x7FFF + ((u >> 16) & 1)) & 0xFFFF0000
    return u.astype(np.uint32).view(np.float32).astype(np.int64)


def _v_index(r):
    if r <= 256:
        return int(r)
    if r <= 512:
        return 256 + int(r - 256) // 2
    if r <= 1024:
        return 384 + int(r - 512) // 4
    return 512 + int(r - 1024) // 8


_BLK_V0 = [128 * c if c < 2 else
           256 + 64 * (c - 2) if c < 4 else
           384 + 32 * (c - 4) if c < 8 else
           512 + 16 * (c - 8) for c in range(NB)]
_BLK_NV = [128 if c < 2 else 80 if c < 4 else 48 if c < 8 else 32
           for c in range(NB)]
_COARSE = ([(r, r, 8) for r in range(8)]
           + [(256 + 2 * r, 256 + r, 4) for r in range(4)]
           + [(512 + 256 * k + 4 * r, 384 + 64 * k + r, 2)
              for k in range(2) for r in range(2)]
           + [(1024 + 256 * k, 512 + 32 * k, 1) for k in range(4)]
           + [(2048, 640, 1)])


def _constants():
    t = np.arange(BK)[None, :]
    f = np.arange(BK)[:, None]
    th = 2.0 * np.pi * ((t * (2 * f + 1)) % 512) / 512.0
    fwd = np.concatenate([np.cos(th), -np.sin(th)], axis=0)
    inv = np.concatenate([np.cos(th).T, -np.sin(th).T], axis=1) / BK
    rpos = _round_positions()
    sel = []
    for c in (2, 4, 8):
        w = np.zeros((2 * BK, _BLK_NV[c]))
        for tt in range(BK):
            w[:, _v_index(rpos[c * BK + tt]) - _BLK_V0[c]] += fwd[:, tt]
        sel.append(w)
        for c2 in range(c, 2 * c):
            for tt in range(BK):
                assert (_v_index(rpos[c2 * BK + tt]) - _BLK_V0[c2]
                        == _v_index(rpos[c * BK + tt]) - _BLK_V0[c])
    for c2 in range(2):
        for tt in range(BK):
            assert rpos[c2 * BK + tt] == c2 * BK + tt
    return fwd, inv, sel


def _cmul(ar, ai, br, bi):
    return ar * br - ai * bi, ar * bi + ai * br


def _layernorm(x):
    m = jnp.mean(x, axis=-1, keepdims=True)
    xc = x - m
    v = jnp.mean(xc * xc, axis=-1, keepdims=True)
    return xc * lax.rsqrt(v + EPS)


def _pk(x):
    return pltpu.bitcast(x, jnp.uint32)


def _upk(x):
    return pltpu.bitcast(x, bf16)


def _dot(a, b):
    return jnp.dot(a, b, preferred_element_type=f32)


def _kernel(x_hbm, are_ref, aim_ref, bre_ref, bim_ref, cre_ref, cim_ref,
            ldt_ref, dsk_ref, w1_hbm, w2_hbm, w3_hbm, w4_hbm,
            fwd_ref, inv_ref, s1_ref, s2_ref, s3_ref,
            out_hbm,
            x_v, w1_v, w2_v, w3_v, w4_v, out_v,
            dt_s, p1_s, p2_s, r_s, kd_s, kf_s, xf_s, xn_s, h_s, z_s, x1_s, ln_s, h3_s, w1_u, w2_u, w3_u, w4_u, pa_s, pb_s,
            flag_s, in_sems, out_sems):
    cp_x = pltpu.make_async_copy(x_hbm.at[0], x_v, in_sems.at[0])
    flag_s[0] = 1

    def wcopies(j, src, dst):
        return [pltpu.make_async_copy(src.at[:, pl.ds(q * 128, 128)],
                                      dst.at[q, pl.ds(0, src.shape[0])],
                                      in_sems.at[1 + 4 * j + q]) for q in range(4)]

    cp_w1 = wcopies(0, w1_hbm, w1_v)
    cp_w2 = wcopies(1, w2_hbm, w2_v)
    cp_w3 = wcopies(2, w3_hbm, w3_v)
    cp_w4 = wcopies(3, w4_hbm, w4_v)
    for cp in [cp_x] + cp_w1 + cp_w2 + cp_w3 + cp_w4:
        cp.start()
    for q in range(4):
        w3_v[q, pl.ds(F, FP - F), :] = jnp.zeros((FP - F, 128), bf16)
        w4_v[q, pl.ds(F, FP - F), :] = jnp.zeros((FP - F, 128), bf16)

    dt_row = jnp.exp(ldt_ref[...].reshape(1, D).astype(f32)).astype(bf16).astype(f32)
    dt_s[...] = jnp.broadcast_to(dt_row, (N, D)).T

    def gen_powers(r0, CH):
        rows = pl.ds(r0, CH)
        dt = dt_s[rows, :]
        ar = dt * are_ref[rows, :].astype(f32)
        ai = dt * aim_ref[rows, :].astype(f32)
        dbr = dt * bre_ref[rows, :].astype(f32)
        dbi = dt * bim_ref[rows, :].astype(f32)
        cbr, cbi = _cmul(cre_ref[rows, :].astype(f32), cim_ref[rows, :].astype(f32),
                         dbr, dbi)

        def put1(r, v):
            p1_s[0, pl.ds(r * PITCH + r0, CH), :] = v[0]
            p1_s[1, pl.ds(r * PITCH + r0, CH), :] = v[1]

        e = jnp.exp(ar)
        l1 = (e * jnp.cos(ai), e * jnp.sin(ai))
        yield
        l2 = _cmul(*l1, *l1)
        l4 = _cmul(*l2, *l2)
        l8 = _cmul(*l4, *l4)
        n1 = l8
        for _ in range(5):
            n1 = _cmul(*n1, *n1)
        q = (cbr, cbi)
        for j in range(NJ):
            p2_s[0, pl.ds(j * PITCH + r0, CH), :] = q[0]
            p2_s[1, pl.ds(j * PITCH + r0, CH), :] = -q[1]
            if j + 1 < NJ:
                q = _cmul(*q, *l8)
            if j in (9, 20, NJ - 1):
                yield
        one = jnp.ones_like(ar)
        zero = jnp.zeros_like(ar)
        put1(0, (one, zero))
        put1(1, l1)
        put1(2, l2)
        put1(3, _cmul(*l2, *l1))
        put1(4, l4)
        put1(5, _cmul(*l4, *l1))
        l6 = _cmul(*l4, *l2)
        put1(6, l6)
        put1(7, _cmul(*l6, *l1))
        put1(8, n1)
        put1(9, _cmul(*n1, *l2))
        put1(10, _cmul(*n1, *l4))
        put1(11, _cmul(*n1, *l6))
        yield
        n2 = _cmul(*n1, *n1)
        put1(12, n2)
        put1(13, _cmul(*n2, *l4))
        n3 = _cmul(*n2, *n1)
        put1(14, n3)
        put1(15, _cmul(*n3, *l4))
        n4 = _cmul(*n2, *n2)
        put1(16, n4)
        put1(17, _cmul(*n4, *n1))
        put1(18, _cmul(*n4, *n2))
        put1(19, _cmul(*n4, *n3))
        put1(20, _cmul(*n4, *n4))
        for r in range(21, NR):
            put1(r, (zero, zero))

    def pow_first(ci, carry):
        for _ in gen_powers(pl.multiple_of(ci * 32, 8), 32):
            pass
        return carry

    with jax.named_scope('sc_pow'):
        lax.fori_loop(0, PW0 // 32, pow_first, 0)

    cp_x.wait()
    for cp in cp_w1:
        cp.wait()
    for q in range(4):
        w1_u[q] = _pk(w1_v[q])
    h_s[pl.ds(0, HPAD), :] = jnp.zeros((HPAD, D), f32)
    h_s[pl.ds(HPAD + L, HPAD), :] = jnp.zeros((HPAD, D), f32)

    def pre_ln(b):
        rows = pl.ds(pl.multiple_of(b * BK, BK), BK)
        xn = _layernorm(x_v[rows, :].astype(f32)).astype(bf16)
        xn_s[rows, :] = xn
        xnn = _layernorm(xn.astype(f32)).astype(bf16)
        for k in range(4):
            pa_s[b % 2, k] = _pk(xn[:, k * 128:(k + 1) * 128])
            pb_s[b % 2, k] = _pk(xnn[:, k * 128:(k + 1) * 128])

    def pre_mm(b, gen):
        r0 = pl.multiple_of(b * BK, BK)
        xnn = jnp.concatenate([_upk(pb_s[b % 2, k]) for k in range(4)], axis=1)
        for q in range(4):
            xf = _dot(fwd_ref[...], _upk(pa_s[b % 2, q]))
            xf_s[b, q, 0:2 * BK, :] = xf
            xf_s[b, q, 2 * BK:3 * BK, :] = xf[0:BK] + xf[BK:2 * BK]
            next(gen, None)
            h = jax.nn.gelu(_dot(xnn, _upk(w1_u[q])), approximate=True)
            h_s[pl.ds(HPAD + r0, BK), pl.ds(q * 128, 128)] = h.astype(bf16).astype(f32)
            if q > 0:
                next(gen, None)

    def pre(b, carry):
        pre_mm(b, iter(()))
        pre_ln(jnp.minimum(b + 1, NB - 1))
        for _ in gen_powers(pl.multiple_of(PW0 + b * PWB, 8), PWB):
            pass
        return carry

    with jax.named_scope('sc_pre'):
        pre_ln(0)
        lax.fori_loop(0, NB, pre, 0, unroll=16)

    lane_blk = lax.broadcasted_iota(jnp.int32, (NR, 128), 1) // NJ

    def group(g, carry):
        p1 = jnp.concatenate([jnp.concatenate(
            [p1_s[ri, pl.ds(dp * 128 + g, NR, stride=PITCH), :] for dp in range(4)], axis=0)
            for ri in range(2)], axis=1)
        p2 = jnp.concatenate([jnp.concatenate(
            [p2_s[ri, pl.ds(dp * 128 + g, NJ, stride=PITCH), :] for dp in range(4)], axis=0)
            for ri in range(2)], axis=1)
        o = lax.dot_general(p1.astype(bf16), p2.astype(bf16),
                            (((1,), (1,)), ((), ())), preferred_element_type=f32)
        r = jnp.where(lane_blk == 0, o[0:NR],
                      jnp.where(lane_blk == 1, o[NR:2 * NR],
                                jnp.where(lane_blk == 2, o[2 * NR:3 * NR],
                                          o[3 * NR:4 * NR])))
        r_s[pl.ds(g, NR, stride=RP), :] = r
        return carry

    with jax.named_scope('sc_grp'):
        lax.fori_loop(0, 128, group, 0, unroll=16)

    for dp in range(4):
        kd_s[dp, pl.ds(648, 8), :] = jnp.zeros((8, 128), f32)
    for r, (_, v0, st) in enumerate(_COARSE):
        t = r_s[pl.ds(r * RP, 128), :].T
        for dp in range(4):
            slab = t[dp * NJ:(dp + 1) * NJ, :]
            if r == 20:
                kd_s[dp, pl.ds(v0, 8), :] = slab[0:8]
            elif st == 1:
                kd_s[dp, pl.ds(v0, NJ), :] = slab
            else:
                kd_s[dp, pl.ds(v0, NJ, stride=st), :] = slab

    sgn = jnp.where(lax.broadcasted_iota(jnp.int32, (BK, 1), 0) % 2 == 0, 1.0, -1.0)
    for dp in range(4):
        prev = None
        ln_ = pl.ds(dp * 128, 128)
        for c in range(NB):
            w = (fwd_ref if c < 2 else s1_ref if c < 4 else s2_ref if c < 8 else s3_ref)[...]
            kf = _dot(w, kd_s[dp, pl.ds(_BLK_V0[c], _BLK_NV[c]), :].astype(bf16))
            kr, ki = kf[0:BK], kf[BK:2 * BK]
            if prev is None:
                kr2, ki2 = kr, ki
            else:
                kr2, ki2 = kr - sgn * prev[1], ki + sgn * prev[0]
            kf_s[c, dp, 0:BK, :] = kr2
            kf_s[c, dp, BK:2 * BK, :] = ki2
            kf_s[c, dp, 2 * BK:3 * BK, :] = kr2 + ki2
            prev = (kr, ki)

    for cp in cp_w2 + cp_w3 + cp_w4:
        cp.wait()
    for q in range(4):
        w2_u[q] = _pk(w2_v[q])
        for j in range(FP // 128):
            w3_u[q, j] = _pk(w3_v[q, pl.ds(j * 128, 128), :])
            w4_u[q, j] = _pk(w4_v[q, pl.ds(j * 128, 128), :])

    out_copies = []
    dsk = dsk_ref[...].reshape(1, D).astype(f32)
    c4 = D // 4
    KB = TP // BK
    ZR = 8
    NI = BK // ZR
    NU = 4 * NI
    NH = FP // 128

    QB = 8

    def zunit(P, u):
        q = u // NI
        r = (u % NI) * ZR
        rs = [pl.ds(pln * BK + r, ZR) for pln in range(3)]
        acc = [None] * QB
        xc = {}
        for c in range(P * QB + QB):
            kk = [kf_s[c, q, rr, :] for rr in rs]
            for k in range(QB):
                b = P * QB + k
                if c > b:
                    continue
                if b - c not in xc:
                    xc[b - c] = [xf_s[b - c, q, rr, :] for rr in rs]
                t = tuple(kv * xv for kv, xv in zip(kk, xc[b - c]))
                acc[k] = t if acc[k] is None else tuple(a + v for a, v in zip(acc[k], t))
        for k in range(QB):
            p1, p2, p3 = acc[k]
            z_s[P * QB + k, q, 0, rs[0], :] = (p1 - p2).astype(bf16)
            z_s[P * QB + k, q, 1, rs[0], :] = (p3 - p1 - p2).astype(bf16)

    def zloop(P):
        for u0 in range(0, NU, ZG):
            @pl.when(flag_s[0] == 1)
            def _(u0=u0):
                for u in range(u0, u0 + ZG):
                    zunit(P, u)

    NM = TP // MS
    for p in range(NP):
        r0 = p * TP
        if (p * KB) % QB == 0:
            zloop(p * KB // QB)
        for m in range(NM):
            rm = r0 + m * MS
            mr = pl.ds(m * MS, MS)
            mh = pl.ds(m * MS // 2, MS // 2)
            hsft = jnp.concatenate([
                h_s[pl.ds(HPAD + rm - 1, MS), 0 * c4:1 * c4],
                h_s[pl.ds(HPAD + rm + 1, MS), 1 * c4:2 * c4],
                h_s[pl.ds(HPAD + rm - 2, MS), 2 * c4:3 * c4],
                h_s[pl.ds(HPAD + rm + 2, MS), 3 * c4:4 * c4]], axis=1).astype(bf16)
            for q in range(4):
                ln_ = pl.ds(q * 128, 128)
                x1_s[mr, ln_] = (xn_s[pl.ds(rm, MS), ln_].astype(f32)
                                 + _dot(hsft, _upk(w2_u[q])))
            ln = _layernorm(x1_s[mr, :]).astype(bf16)
            for k in range(4):
                ln_s[k, mh, :] = _pk(ln[:, k * 128:(k + 1) * 128])
        for j in range(NH):
            for m in range(NM):
                mh = pl.ds(m * MS // 2, MS // 2)
                acc = None
                for k in range(4):
                    t = lax.dot_general(_upk(ln_s[k, mh, :]), _upk(w3_u[k, j]),
                                        (((1,), (1,)), ((), ())), preferred_element_type=f32)
                    acc = t if acc is None else acc + t
                h3_s[j, mh, :] = _pk(jax.nn.gelu(acc, approximate=True).astype(bf16))
        for q in range(4):
            ln_ = pl.ds(q * 128, 128)
            for m in range(NM):
                mr = pl.ds(m * MS, MS)
                mh = pl.ds(m * MS // 2, MS // 2)
                rows = pl.ds(r0 + m * MS, MS)
                o2 = x1_s[mr, ln_]
                for j in range(NH):
                    o2 = o2 + _dot(_upk(h3_s[j, mh, :]), _upk(w4_u[q, j]))
                if MS == BK:
                    y = (_dot(inv_ref[0], z_s[p * KB + m, q, 0])
                         + _dot(inv_ref[1], z_s[p * KB + m, q, 1]))
                else:
                    y = jnp.concatenate([_dot(inv_ref[0], z_s[p * KB + k, q, 0])
                                         + _dot(inv_ref[1], z_s[p * KB + k, q, 1])
                                         for k in range(KB)], axis=0)
                hh = 0.5 * o2
                gate = hh + hh * jnp.tanh(hh)
                s = y + xn_s[rows, ln_].astype(f32) * dsk[:, q * 128:(q + 1) * 128]
                res = x_v[rows, ln_].astype(f32) + s * gate
                out_v[rows, ln_] = res.astype(bf16)
        cp = pltpu.make_async_copy(out_v.at[pl.ds(r0, TP), :],
                                   out_hbm.at[0, pl.ds(r0, TP), :], out_sems.at[p])
        cp.start()
        out_copies.append(cp)
    for cp in out_copies:
        cp.wait()


@jax.jit
def pallas_recurrent_scan__ssm_conv_s4__mixer_s_mlp__prompt_kernel(
    A_u: jax.Array,
    A_A_re: jax.Array,
    A_A_im: jax.Array,
    A_B_re: jax.Array,
    A_B_im: jax.Array,
    A_C_re: jax.Array,
    A_C_im: jax.Array,
    A_log_dt: jax.Array,
    A_Dskip: jax.Array,
    B_x: jax.Array,
    B_w1: jax.Array,
    B_w2: jax.Array,
    B_w3: jax.Array,
    B_w4: jax.Array,
):
    assert A_u.shape == (1, L, D) and A_A_re.shape == (D, N)
    assert A_u.dtype == bf16 and A_A_re.dtype == bf16
    assert B_w3.shape == (D, F)
    fwd, inv, sel = _constants()
    inv = np.stack([inv[:, :BK], inv[:, BK:]])
    consts = [jnp.asarray(c, dtype=bf16) for c in (fwd, inv, *sel)]

    vmem = pl.BlockSpec(memory_space=pltpu.VMEM)
    hbm = pl.BlockSpec(memory_space=pltpu.HBM)
    return pl.pallas_call(
        _kernel,
        out_shape=jax.ShapeDtypeStruct((1, L, D), bf16),
        in_specs=[hbm] + [vmem] * 8 + [hbm] * 4 + [vmem] * 5,
        out_specs=hbm,
        scratch_shapes=[
            pltpu.VMEM((L, D), bf16),
            pltpu.VMEM((4, D, 128), bf16),
            pltpu.VMEM((4, D, 128), bf16),
            pltpu.VMEM((4, FP, 128), bf16),
            pltpu.VMEM((4, FP, 128), bf16),
            pltpu.VMEM((L, D), bf16),
            pltpu.VMEM((D, N), f32),
            pltpu.VMEM((2, NR * PITCH, N), f32),
            pltpu.VMEM((2, NJ * PITCH, N), f32),
            pltpu.VMEM((NR * RP, 128), f32),
            pltpu.VMEM((4, NV, 128), f32),
            pltpu.VMEM((NB, 4, 3 * BK, 128), f32),
            pltpu.VMEM((NB, 4, 3 * BK, 128), f32),
            pltpu.VMEM((L, D), bf16),
            pltpu.VMEM((L + 2 * HPAD, D), f32),
            pltpu.VMEM((NB, 4, 2, BK, 128), bf16),
            pltpu.VMEM((TP, D), f32),
            pltpu.VMEM((4, TP // 2, 128), jnp.uint32),
            pltpu.VMEM((FP // 128, TP // 2, 128), jnp.uint32),
            pltpu.VMEM((4, D // 2, 128), jnp.uint32),
            pltpu.VMEM((4, D // 2, 128), jnp.uint32),
            pltpu.VMEM((4, FP // 128, 64, 128), jnp.uint32),
            pltpu.VMEM((4, FP // 128, 64, 128), jnp.uint32),
            pltpu.VMEM((2, 4, 64, 128), jnp.uint32),
            pltpu.VMEM((2, 4, 64, 128), jnp.uint32),
            pltpu.SMEM((1,), jnp.int32),
            pltpu.SemaphoreType.DMA((17,)),
            pltpu.SemaphoreType.DMA((NP,)),
        ],
        compiler_params=pltpu.CompilerParams(vmem_limit_bytes=110 * 1024 * 1024),
    )(A_u, A_A_re, A_A_im, A_B_re, A_B_im, A_C_re, A_C_im,
      A_log_dt, A_Dskip,
      B_w1, B_w2, B_w3.T, B_w4, *consts)
```
